```python
import os as _os
_os.environ.setdefault('JAX_PLATFORMS', 'cpu')
import jax
import jax.numpy as jnp

def _softmax(x, axis=-1):
    return jax.nn.softmax(x, axis=axis)

def _gelu(x):
    return jax.nn.gelu(x, approximate=True)

def _silu(x):
    return jax.nn.silu(x)

def _sigmoid(x):
    return jax.nn.sigmoid(x)

def _layernorm(x, axis=-1, eps=1e-05):
    m = jnp.mean(x, axis=axis, keepdims=True)
    v = jnp.var(x, axis=axis, keepdims=True)
    return (x - m) / jnp.sqrt(v + eps)

def _scatter_add(tgt, idx, src, axis=0):
    return tgt.at[idx].add(src)

def _segment_sum(src, seg, n):
    return jax.ops.segment_sum(src, seg, n)

class _Rng:

    def __init__(self, key):
        self._k = key

    def _next(self):
        self._k, sub = jax.random.split(self._k)
        return sub

    def normal(self, shape):
        return jax.random.normal(self._next(), shape, dtype=jnp.bfloat16)

    def randint(self, lo, hi, shape):
        return jax.random.randint(self._next(), shape, lo, hi, dtype=jnp.int32)

    def uniform(self, shape, lo=0.0, hi=1.0):
        return jax.random.uniform(self._next(), shape, jnp.bfloat16, lo, hi)

    def permutation(self, n):
        return jax.random.permutation(self._next(), n)
kernel_name = 'adaLN_cond__mha_block__geglu_ffn__prompt'

def setup_inputs():
    _rng = _Rng(jax.random.key(int.from_bytes(__import__("os").urandom(4), "little")))
    _w = lambda a: (lambda t: t.astype(jnp.bfloat16) if jnp.issubdtype(t.dtype, jnp.floating) else t)(jnp.asarray(a))

    def _A_setup():
        B, S, D, H = (1, 2048, 512, 32)
        return {'x': _w((lambda *s: _rng.normal(s) * 0.05)(B, S, D)), 'wqkv': _w((lambda *s: _rng.normal(s) * 0.05)(D, 3 * D)), 'wo': _w((lambda *s: _rng.normal(s) * 0.05)(D, D))}
    _A_in = _A_setup()

    def _B_setup():
        B, S, D, F = (1, 2048, 512, 1376)
        return {'x': _w((lambda *s: _rng.normal(s) * 0.05)(B, S, D)), 'w_gate': _w((lambda *s: _rng.normal(s) * 0.05)(D, F)), 'w_up': _w((lambda *s: _rng.normal(s) * 0.05)(D, F)), 'w_down': _w((lambda *s: _rng.normal(s) * 0.05)(F, D))}
    _B_in = _B_setup()
    return {'A_x': _A_in['x'], 'A_wqkv': _A_in['wqkv'], 'A_wo': _A_in['wo'], 'B_x': _B_in['x'], 'B_w_gate': _B_in['w_gate'], 'B_w_up': _B_in['w_up'], 'B_w_down': _B_in['w_down'], 'c': _w((lambda *s: _rng.normal(s) * 0.05)(1, 512) * 8.0), 'w_mod': _w((lambda *s: _rng.normal(s) * 0.05)(512, 6 * 512) * 512 ** (-0.5) * 8.0)}

def reference(A_x, A_wqkv, A_wo, B_x, B_w_gate, B_w_up, B_w_down, c, w_mod):

    def _A_ref(x, wqkv, wo):
        B, S, D = x.shape
        H = 32
        Dh = D // H
        qkv = (lambda x, *d: x.transpose(*d))((x @ wqkv).reshape(B, S, 3, H, Dh), 2, 0, 3, 1, 4)
        q, k, v = (qkv[0], qkv[1], qkv[2])
        scores = jnp.einsum('bhqd,bhkd->bhqk', q, k) * Dh ** (-0.5)
        p = _softmax(scores, axis=-1)
        o = jnp.einsum('bhqk,bhkd->bhqd', p, v)
        return (lambda x, *d: x.transpose(*d))(o, 0, 2, 1, 3).reshape(B, S, D) @ wo

    def _B_ref(x, w_gate, w_up, w_down):
        return _gelu(x @ w_gate) * (x @ w_up) @ w_down
    x = A_x
    mod = (_silu(c) @ w_mod).reshape(c.shape[0], 6, 1, -1)
    sa, ca, ga, sb, cb, gb = (mod[:, 0].copy(), mod[:, 1].copy(), mod[:, 2].copy(), mod[:, 3].copy(), mod[:, 4].copy(), mod[:, 5].copy())
    h = _layernorm(x, axis=-1) * (1 + ca) + sa
    x = x + ga * _A_ref(h, A_wqkv, A_wo)
    h = _layernorm(x, axis=-1) * (1 + cb) + sb
    x = x + gb * _B_ref(h, B_w_gate, B_w_up, B_w_down)
    return x
```

```python
import functools

import jax
import jax.numpy as jnp
import numpy as np
from jax import lax
from jax.experimental import pallas as pl
from jax.experimental.pallas import tpu as pltpu

S, D, H, DH, F = 2048, 512, 32, 16, 1376
EPS = 1e-5
LOG2E = float(np.log2(np.e))
f32, bf16, i32 = jnp.float32, jnp.bfloat16, jnp.int32
bc = pltpu.bitcast

CFG = dict(pat="1", ldelay=12, head=7, tail=7, kgrp=4, kpin=0, tb1=256, tb3=512, hpi=1,
           lgate="rot", chains=1, ut=1, name="fused", force_slow=0, fchunk=128)

TQ, CK = 512, 128
NQ, NC, NT = S // TQ, S // CK, TQ // 128
HS = S // 16 + 2 * NC
SAFE = 2.0 ** 60


def _dot(a, b):
    return jnp.dot(a, b, preferred_element_type=f32)


def _dot_nt(a, b):
    return lax.dot_general(a, b, (((1,), (1,)), ((), ())), preferred_element_type=f32)


def build(cfg):
    a = type("A", (), {**CFG, **cfg})
    pat = [int(x) for x in a.pat]
    NVB = [pat[c % len(pat)] for c in range(NC)]
    VOFF = [int(x) for x in np.concatenate([[0], np.cumsum(NVB)])]
    NVT = VOFF[-1]
    A_W = H * HS
    W_L, W_ACC, W_LC, W_PC, W_PV = 0, 4, 12, 16, 80
    PVS = NVT * 2 * 16
    A_N = A_W + W_PV + 2 * PVS
    TB1, TB3 = a.tb1, a.tb3
    NB1, NB3 = S // TB1, S // TB3

    def vblocks(c):
        return list(range(8 - NVB[c], 8))

    def kernel(x_h, wqkv_h, wo_h, wgt_h, wut_h, wd_h, c_h, wmod_h, out_h,
               x_v, wqkv_v, wo_v, wgt_v, wut_v, wd_v, c_v, wmod_v,
               wqt_s, wvt_s, wot_s, wdt_s, h_s, col_s,
               ar, qt_s, qf_s, kf_s, kb_s, ot_s, rng_s,
               x1_s, h2_s, act_s, o_v, sem, osem):
        cps = {}

        def start(name, src, dst):
            cps[name] = pltpu.make_async_copy(src, dst, sem.at[len(cps)])
            cps[name].start()

        start("c", c_h, c_v)
        start("mod0", wmod_h.at[:, pl.ds(0, 2 * D)], wmod_v.at[:, pl.ds(0, 2 * D)])
        start("x0", x_h.at[pl.ds(0, TB1)], x_v.at[pl.ds(0, TB1)])
        start("wk", wqkv_h.at[:, pl.ds(D, D)], wqkv_v.at[:, pl.ds(D, D)])
        start("wq", wqkv_h.at[:, pl.ds(0, D)], wqkv_v.at[:, pl.ds(0, D)])
        start("x1", x_h.at[pl.ds(TB1, S - TB1)], x_v.at[pl.ds(TB1, S - TB1)])
        start("wv", wqkv_h.at[:, pl.ds(2 * D, D)], wqkv_v.at[:, pl.ds(2 * D, D)])
        start("mod1", wmod_h.at[:, pl.ds(2 * D, 4 * D)], wmod_v.at[:, pl.ds(2 * D, 4 * D)])
        start("wo", wo_h, wo_v)
        start("wd", wd_h, wd_v)
        start("wg", wgt_h, wgt_v)
        start("wu", wut_h, wut_v)

        cps["c"].wait()
        cf = c_v[...].astype(f32)
        sc = jnp.broadcast_to(cf / (1.0 + jnp.exp(-cf)), (16, D)).astype(bf16)

        def modvec(i):
            m = _dot(sc, wmod_v[:, i * D:(i + 1) * D])[0:8]
            return m.astype(bf16).astype(f32)

        cps["mod0"].wait()
        sa = modvec(0)[0:1]
        ca1 = (1.0 + modvec(1)).astype(bf16).astype(f32)[0:1]

        def ln_rows(r):
            x = x_v[r, :].astype(f32)
            xc = x - jnp.sum(x, axis=1, keepdims=True) * (1.0 / D)
            var = jnp.sum(xc * xc, axis=1, keepdims=True) * (1.0 / D)
            h_s[r, :] = (xc * lax.rsqrt(var + EPS) * ca1 + sa).astype(bf16)

        def k_proj(b):
            h = h_s[b * TB1:(b + 1) * TB1, :]
            k = bc(_dot(h, wqkv_v[:, D:2 * D]).astype(bf16), i32)
            for g in range(4):
                for j in range(8):
                    hd = g * 8 + j
                    kk = k[:, g * 128:(g + 1) * 128]
                    if j:
                        kk = pltpu.roll(kk, 128 - 16 * j, 1)
                    for i in range(TB1 // 16):
                        blk = b * (TB1 // 16) + i
                        c, bb = blk // 8, blk % 8
                        ar[hd * HS + blk] = kk[i * 8:(i + 1) * 8]
                        if bb in vblocks(c):
                            kf_s[hd, VOFF[c] + vblocks(c).index(bb)] = kk[i * 8:(i + 1) * 8]

        def q_proj(b):
            h = h_s[b * TB1:(b + 1) * TB1, :]
            q = _dot_nt(bc(wqt_s[...], bf16), h) * (DH ** -0.5 * LOG2E)
            qp = bc(q.astype(bf16), i32)
            for hd in range(H):
                qf_s[hd, :, b * TB1:(b + 1) * TB1] = q[hd * 16:(hd + 1) * 16]
                qt_s[hd, :, b * TB1:(b + 1) * TB1] = qp[hd * 8:(hd + 1) * 8]

        def v_proj(b):
            h = h_s[b * TB1:(b + 1) * TB1, :]
            v = bc(_dot_nt(bc(wvt_s[...], bf16), h), i32)
            for t in range(TB1 // 128):
                for r in range(2 * H):
                    ar[(r // 2) * HS + S // 16 + 2 * (b * (TB1 // 128) + t) + r % 2] = (
                        v[r * 8:(r + 1) * 8, t * 128:(t + 1) * 128])

        cps["x0"].wait()
        ln_rows(pl.ds(0, TB1))
        cps["wk"].wait()
        k_proj(0)
        cps["wq"].wait()
        cps["x1"].wait()
        wqt_s[...] = bc(wqkv_v[:, 0:D].T, i32)
        for b in range(NB1):
            if b + 1 < NB1:
                ln_rows(pl.ds((b + 1) * TB1, TB1))
            q_proj(b)
            if b + 1 < NB1:
                k_proj(b + 1)
        for name in ("wv", "mod1", "wo", "wd"):
            cps[name].wait()
        wvt_s[...] = bc(wqkv_v[:, 2 * D:3 * D].T, i32)

        items = [(qb, c) for qb in range(NQ) for c in range(NC)]
        units = [(g, t) for g in range(NVT * 2) for t in range(0, S // 128, a.ut)]

        def make_kb(hd, W, j, d):
            x = jnp.broadcast_to(kf_s[hd, j][:, d:d + 1], (8, 128))
            kb_s[j, d] = bc(x, bf16).astype(f32)
            if W is not None and a.kpin:
                W[W_L] = x

        def vunit(hd, dst, u):
            g, t0 = u
            acc = [{} for _ in range(a.chains)]
            for d in range(16):
                kb = kb_s[g // 2, d, (g % 2) * 8:(g % 2 + 1) * 8, :]
                for t in range(t0, t0 + a.ut):
                    pr = kb * qf_s[hd, d:d + 1, t * 128:(t + 1) * 128]
                    A = acc[d % a.chains]
                    A[t] = pr if t not in A else A[t] + pr
            for t in acc[0]:
                s = acc[0][t]
                for A in acc[1:]:
                    s = s + A[t]
                dst[g * 16 + t] = bc(jnp.exp2(s), i32)

        def tile(ref, fn, rows):
            return jnp.concatenate(
                [jnp.concatenate([bc(ref[fn(r, t)], f32) for t in range(NT)], axis=1)
                 for r in range(rows)], axis=0)

        def untile(x, ref, fn):
            for r in range(x.shape[0] // 8):
                for t in range(NT):
                    ref[fn(r, t)] = bc(x[r * 8:(r + 1) * 8, t * 128:(t + 1) * 128], i32)

        def pv(A, c, p):
            vt = bc(jnp.concatenate([A[S // 16 + 2 * c], A[S // 16 + 2 * c + 1]], axis=0), f32)
            return _dot(vt, p)

        def finish(hd, qb, l, acc):
            lt = jnp.broadcast_to(l.sum(axis=0, keepdims=True), (8, TQ))
            r = 1.0 / lt
            ot_s[hd, :, qb * TQ:(qb + 1) * TQ] = bc((acc * r[0:1]).astype(bf16), i32)
            rng_s[...] += (lt + r) + (jnp.abs(acc[:8]) + jnp.abs(acc[8:]))

        def carried(hp, W):
            p = tile(W, lambda r, t: W_PC + r * NT + t, 16)
            acc = pv(ar.at[pl.ds(hp * HS, HS)], NC - 1, p) + tile(W, lambda r, t: W_ACC + r * NT + t, 2)
            finish(hp, NQ - 1, tile(W, lambda r, t: W_LC + t, 1), acc)

        if units:
            for d in range(16):
                for j in range(NVT):
                    make_kb(0, None, j, d)
            dst0 = ar.at[pl.ds(A_W + W_PV, PVS)]
        for b in range(NB1):
            v_proj(b)
            for u in units[b * len(units) // NB1:(b + 1) * len(units) // NB1]:
                vunit(0, dst0, u)
        if units:
            for d in range(16):
                for j in range(NVT):
                    make_kb(1, None, j, d)
        for i in range(2, 6):
            m = modvec(i)
            if i == 4:
                m = (1.0 + m).astype(bf16).astype(f32)
            col_s[i - 2] = jnp.broadcast_to(m[0:1], (128, D)).T
        wot_s[...] = bc(wo_v[...].T, i32)
        for j in range(0, F, 128):
            w = min(128, F - j)
            wdt_s[:, j:j + w] = bc(wd_v[j:j + w, :].T, i32)
        for r in range(W_PV):
            ar[A_W + r] = bc(jnp.ones((8, 128), f32), i32)
        rng_s[...] = jnp.zeros_like(rng_s)

        def body(it, carry):
            h0 = it * a.hpi
            W = ar.at[pl.ds(A_W + (it >> 8), W_PV)]
            nsl = sum(8 - NVB[c] + 1 for qb, c in items)
            work = []
            for u in range(a.hpi):
                hd = h0 + u
                hn = jnp.minimum(hd + 1, H - 1)
                h2 = jnp.minimum(hd + 2, H - 1)
                if units:
                    dst = ar.at[pl.ds(A_W + W_PV + ((hd + 1) & 1) * PVS, PVS)]
                for k, x in enumerate(units):
                    work.append((u + (k + 1) / len(units), functools.partial(vunit, hn, dst, x)))
                G = a.kgrp
                kbs = [(j0 + j, d if (j0 // G) % 2 == 0 else 15 - d)
                       for j0 in range(0, NVT, G) for d in range(16) for j in range(min(G, NVT - j0))]
                for k, (j, d) in enumerate(kbs):
                    work.append((u + min(1.0 + 1e-6, (k + 16 * G + 0.1) / len(kbs)),
                                 functools.partial(make_kb, h2, W, j, d)))
            work.sort(key=lambda w: w[0])
            P, L, ACC = {}, {}, {}
            st = dict(slot=0)
            lq = []

            def slot():
                st["slot"] += 1
                fr = a.hpi * (st["slot"] - a.head) / (nsl * a.hpi + a.tail - a.head)
                while work and work[0][0] <= fr:
                    work.pop(0)[1]()
                while lq and lq[0][0] + a.ldelay <= st["slot"]:
                    sl, src = lq.pop(0)
                    if a.lgate == "all":
                        untile(src, W, lambda r, t: W_L + t)
                    elif a.lgate == "rot":
                        t = sl % NT
                        W[W_L + t] = bc(src[:, t * 128:(t + 1) * 128], i32)

            def addl(key, p):
                l = L.get(key)
                l = p[8:] if l is None else l + p[8:]
                L[key] = l + p[:8]

            def fetch(u, i):
                qb, c = items[i]
                for j, b in list(enumerate(vblocks(c)))[::-1]:
                    P[u, i, b] = tile(SRC[u], lambda r, t: ((VOFF[c] + j) * 2 + r) * 16 + qb * NT + t, 2)
                    addl((u, qb), P[u, i, b])

            def gather(u, i):
                return jnp.concatenate([P.pop((u, i, b)) for b in range(8)], axis=0)

            def retire(u, i):
                qb, c = items[i]
                slot()
                d = pv(AH[u], c, gather(u, i))
                ACC[u, qb] = d if (u, qb) not in ACC else d + ACC[u, qb]
                if c == NC - 1:
                    finish(h0 + u, qb, L[u, qb], ACC[u, qb])

            prev = None
            AH = [ar.at[pl.ds((h0 + u) * HS, HS)] for u in range(a.hpi)]
            if units:
                SRC = [ar.at[pl.ds(A_W + W_PV + ((h0 + u + 2) & 1) * PVS, PVS)] for u in range(a.hpi)]
            for u in range(a.hpi):
                hd = h0 + u
                for i, (qb, c) in enumerate(items):
                    order = [b for b in range(8) if b not in vblocks(c)][::-1]
                    qm = bc(qt_s[hd, :, qb * TQ:(qb + 1) * TQ], bf16)
                    ks, sls = [], []
                    for b in order:
                        slot()
                        sls.append(st["slot"])
                        ks.append(AH[u][c * 8 + b])
                    s = _dot(bc(jnp.concatenate(ks, axis=0), bf16)[:, 0:16], qm)
                    if prev is None:
                        slot()
                        carried(jnp.maximum(h0 - 1, 0), W)
                    else:
                        retire(*prev)
                    prev = (u, i)
                    fetch(u, i)
                    for k, b in enumerate(order):
                        p = jnp.exp2(s[k * 16:(k + 1) * 16])
                        P[u, i, b] = p
                        addl((u, qb), p)
                        lq.append((sls[k], L[u, qb]))
            p = gather(*prev)
            for r in range(15, -1, -1):
                untile(p[r * 8:(r + 1) * 8], W, lambda _, t: W_PC + r * NT + t)
                if r % 2 == 0 and work:
                    work.pop(0)[1]()
            while work:
                work.pop(0)[1]()
            untile(ACC[prev[0], NQ - 1], W, lambda r, t: W_ACC + r * NT + t)
            untile(L[prev[0], NQ - 1], W, lambda r, t: W_LC + t)
            return carry

        lax.fori_loop(0, H // a.hpi, body, 0)
        carried(H - 1, ar.at[pl.ds(A_W, W_PV)])

        bad = jnp.sum(jnp.where(rng_s[...] < SAFE, 0, 1)) + a.force_slow

        @pl.when(bad > 0)
        def _():
            def slow(i, carry):
                hd, qb = i // NQ, i % NQ
                A = ar.at[pl.ds(hd * HS, HS)]
                cols = pl.ds(pl.multiple_of(qb * TQ, TQ), TQ)
                k = bc(A[0:S // 16].reshape(S // 2, 128), bf16)[:, 0:16]
                s = _dot(k, bc(qt_s[hd, :, cols], bf16))
                p = jnp.exp2(s - jnp.max(s, axis=0, keepdims=True))
                acc = pv(A, 0, p[0:CK])
                for c in range(1, NC):
                    acc = pv(A, c, p[c * CK:(c + 1) * CK]) + acc
                ot_s[hd, :, cols] = bc((acc / jnp.sum(p, axis=0, keepdims=True)).astype(bf16), i32)
                return carry

            lax.fori_loop(0, H * NQ, slow, 0)

        cps["wg"].wait()
        cps["wu"].wait()

        def col(i):
            return jnp.concatenate([col_s[i]] * (TB3 // 128), axis=1)

        def pre(b, slot_):
            cols = pl.ds(pl.multiple_of(b * TB3, TB3), TB3)
            o = bc(ot_s[:, :, cols].reshape(D // 2, TB3), bf16)
            x1 = x_v[cols, :].T.astype(f32) + col(0) * _dot(bc(wot_s[...], bf16), o)
            x1_s[slot_] = x1
            xc = x1 - jnp.sum(x1, axis=0, keepdims=True) * (1.0 / D)
            var = jnp.sum(xc * xc, axis=0, keepdims=True) * (1.0 / D)
            h2_s[slot_] = bc((xc * lax.rsqrt(var + EPS) * col(2) + col(1)).astype(bf16), i32)

        def gate_up(slot_):
            for j in range(0, F, a.fchunk):
                w = min(a.fchunk, F - j)
                lhs = jnp.concatenate(
                    [r[i:i + 16, :] for i in range(j, j + w, 16) for r in (wgt_v, wut_v)], axis=0)
                gu = _dot(lhs, bc(h2_s[slot_], bf16))
                for i in range(w // 16):
                    g, up = gu[i * 32:i * 32 + 16], gu[i * 32 + 16:i * 32 + 32]
                    th = jnp.tanh(g * (0.7978845608028654 + (0.7978845608028654 * 0.044715) * (g * g)))
                    hg = 0.5 * g
                    act_s[j // 2 + i * 8:j // 2 + (i + 1) * 8, :] = bc(((hg + hg * th) * up).astype(bf16), i32)

        def down(slot_):
            y = _dot(bc(wdt_s[...], bf16), bc(act_s[...], bf16))
            return (x1_s[slot_] + col(3) * y).astype(bf16).T

        def out_copy(b):
            rows = pl.ds(pl.multiple_of(b * TB3, TB3), TB3)
            return pltpu.make_async_copy(o_v.at[rows], out_h.at[rows], osem.at[b])

        pre(0, 0)
        for b in range(NB3):
            gate_up(b % 2)
            if b + 1 < NB3:
                pre(b + 1, (b + 1) % 2)
            o_v[b * TB3:(b + 1) * TB3, :] = down(b % 2)
            out_copy(b).start()
        for b in range(NB3):
            out_copy(b).wait()

    V = pltpu.VMEM
    scratch = [
        V((S, D), bf16), V((D, 3 * D), bf16), V((D, D), bf16), V((F, D), bf16), V((F, D), bf16),
        V((F, D), bf16), V((1, D), bf16), V((D, 6 * D), bf16),
        V((D // 2, D), i32), V((D // 2, D), i32), V((D // 2, D), i32), V((D // 2, F), i32),
        V((S, D), bf16), V((4, D, 128), f32),
        V((A_N, 8, 128), i32), V((H, 8, S), i32), V((H, 16, S), f32),
        V((H, max(NVT, 1), 8, 128), i32), V((max(NVT, 1), 16, 16, 128), f32),
        V((H, 8, S), i32), V((8, TQ), f32),
        V((2, D, TB3), f32), V((2, D // 2, TB3), i32), V((F // 2, TB3), i32), V((S, D), bf16),
        pltpu.SemaphoreType.DMA((12,)), pltpu.SemaphoreType.DMA((NB3,)),
    ]

    def run(A_x, A_wqkv, A_wo, B_x, B_w_gate, B_w_up, B_w_down, c, w_mod):
        del B_x
        hbm = pl.BlockSpec(memory_space=pltpu.HBM)
        out = pl.pallas_call(
            kernel,
            out_shape=jax.ShapeDtypeStruct((S, D), bf16),
            in_specs=[hbm] * 8,
            out_specs=hbm,
            scratch_shapes=scratch,
            name=a.name,
            compiler_params=pltpu.CompilerParams(vmem_limit_bytes=110 << 20),
        )(A_x.reshape(S, D), A_wqkv, A_wo, B_w_gate.T, B_w_up.T, B_w_down, c, w_mod)
        return out.reshape(1, S, D)

    return run


@jax.jit
def pallas_adaLN_cond__mha_block__geglu_ffn__prompt_kernel(
    A_x, A_wqkv, A_wo, B_x, B_w_gate, B_w_up, B_w_down, c, w_mod
):
    return build({})(A_x, A_wqkv, A_wo, B_x, B_w_gate, B_w_up, B_w_down, c, w_mod)
```

```python
import functools

import jax
import jax.numpy as jnp
import numpy as np
from jax import lax
from jax.experimental import pallas as pl
from jax.experimental.pallas import tpu as pltpu

S, D, H, DH, F = 2048, 512, 32, 16, 1376
EPS = 1e-5
Q_SCALE = DH ** -0.5 * float(np.log2(np.e))
SAFE = 2.0 ** 60
f32, bf16, i32 = jnp.float32, jnp.bfloat16, jnp.int32
bc = pltpu.bitcast

TQ, CK = 512, 128
NQ, NC, NT = S // TQ, S // CK, TQ // 128
N_VPU = [2, 1, 1, 1] * (NC // 4)
VPU_BLOCKS = [c * 8 + b for c in range(NC) for b in range(8 - N_VPU[c], 8)]
MXU_BLOCKS = [c * 8 + b for c in range(NC) for b in range(7 - N_VPU[c], -1, -1)]
NV = len(VPU_BLOCKS)
SEGMENT = [int(n) for n in np.cumsum([0, 8, 7, 6, 7, 7, 7, 6, 7, 7, 7, 6, 7, 7, 7, 6, 6])]
LEAD, TRAIL, SUM_DELAY, SCORE_DELAY = 7, 2, 11, 9

K_ROWS, P_ROWS = S // 8, NV * NQ * 32
W_PACE, W_ACC, W_SUM, W_SCORE, W_ROWS = 0, 8, 24, 32, 160
A_V = H // 2 * K_ROWS
A_W = A_V + NQ * D
A_P = A_W + W_ROWS
A_END = A_P + 2 * P_ROWS

TK = 256
TB = 512
NB = S // TB
HD, HT = D // 2, TB // 2
NR = HD // 16
FS = 1280
G1, G2 = 24, 56


def _dot(a, b):
    return jnp.dot(a, b, preferred_element_type=f32)


def _dot_nt(a, b):
    return lax.dot_general(a, b, (((1,), (1,)), ((), ())), preferred_element_type=f32)


def _aligned(start, size, multiple=8):
    return pl.ds(start if isinstance(start, int) else pl.multiple_of(start, multiple), size)


def _tile(i, n=1):
    return slice(i * 128, (i + n) * 128)


def _left_operands(a11, a12, a21, a22):
    f = [x.astype(f32) for x in (a11, a12, a21, a22)]
    ops = [(f[0] + f[3]).astype(bf16), (f[2] + f[3]).astype(bf16), a11, a22,
           (f[0] + f[1]).astype(bf16), (f[2] - f[0]).astype(bf16), (f[1] - f[3]).astype(bf16)]
    return [bc(x, i32) for x in ops]


def _right_operands(b11, b12, b21, b22):
    return [b11 + b22, b11, b12 - b22, b21 - b11, b22, b11 + b12, b21 + b22]


def _strassen(product, done=lambda i, j, c: c):
    m1 = product(0)
    m2 = product(1)
    c22 = m1 - m2
    m3 = product(2)
    c22 = c22 + m3
    m5 = product(4)
    c12 = done(0, 1, m3 + m5)
    c11 = m1 - m5
    c22 = done(1, 1, product(5, c22))
    m4 = product(3)
    c21 = done(1, 0, m2 + m4)
    c11 = c11 + m4
    c11 = done(0, 0, product(6, c11))
    return c11, c12, c21, c22


def _geglu(g, up):
    k = float(np.sqrt(2.0 / np.pi))
    th = jnp.tanh(g * (k + (k * 0.044715) * (g * g)))
    hg = 0.5 * g
    return (hg + hg * th) * up


class _Agenda:
    def __init__(self):
        self.now, self.todo = 0, []

    def add(self, fns, start, span):
        for k, fn in enumerate(fns):
            self.todo.append((self.now + start + span * (k + 1) / len(fns), fn))
        self.todo.sort(key=lambda w: w[0])

    def tick(self, *args):
        self.now += 1
        while self.todo and self.todo[0][0] <= self.now:
            self.todo.pop(0)[1](*args)

    def flush(self):
        while self.todo:
            self.todo.pop(0)[1]()


def _kernel(x_h, wqkv_h, wo_h, wgt_h, wut_h, wd_h, c_h, wmod_h, out_h,
            att_s, kb_s, kb_last_s, qt_s, qf_s, qs_s, kf_s, acc_s, l_s, r_s, range_s,
            h_s, wq_s, wv_s, so_s, sg_s, sd_s, x1_s,
            x_v, wqkv_v, wo_v, wgu_v, wd_v, wmod_v, o_v, col_s, wt_s, wdt_s, c_v, sem):
    groups = {}

    def start(name, src, dst):
        group = groups.setdefault(name, [])
        group.append(pltpu.make_async_copy(src, dst, sem.at[list(groups).index(name)]))
        group[-1].start()

    def wait(name):
        for copy in groups[name]:
            copy.wait()

    def start_gate_up(name, i0, i1):
        rows = pl.ds(i0 * 16, (i1 - i0) * 16)
        start(name, wgt_h.at[rows], wgu_v.at[0, rows])
        start(name, wut_h.at[rows], wgu_v.at[1, rows])

    start("x0", c_h, c_v)
    start("x0", x_h.at[pl.ds(0, 2 * TK)], x_v.at[pl.ds(0, 2 * TK)])
    start("mod", wmod_h.at[:, pl.ds(0, 2 * D)], wmod_v.at[:, pl.ds(0, 2 * D)])
    start("wk", wqkv_h.at[:, pl.ds(D, D)], wqkv_v.at[:, pl.ds(D, D)])
    start("wq", wqkv_h.at[:, pl.ds(0, D)], wqkv_v.at[:, pl.ds(0, D)])
    start("x1", x_h.at[pl.ds(2 * TK, 3 * TK)], x_v.at[pl.ds(2 * TK, 3 * TK)])
    start("x2", x_h.at[pl.ds(5 * TK, 3 * TK)], x_v.at[pl.ds(5 * TK, 3 * TK)])
    start_gate_up("x2", 0, G1)
    start("wv", wqkv_h.at[:, pl.ds(2 * D, D)], wqkv_v.at[:, pl.ds(2 * D, D)])
    start("wv", wo_h, wo_v)
    start("wv", wd_h, wd_v.at[pl.ds(0, F)])
    start_gate_up("wv", G1, G2)
    start_gate_up("rest", G2, F // 16)
    start("rest", wmod_h.at[:, pl.ds(2 * D, 4 * D)], wmod_v.at[:, pl.ds(2 * D, 4 * D)])

    def normed(r0, n):
        x = x_v[r0:r0 + n, :].astype(f32)
        xc = x - jnp.sum(x, axis=1, keepdims=True) * (1.0 / D)
        var = jnp.sum(xc * xc, axis=1, keepdims=True) * (1.0 / D)
        return xc * lax.rsqrt(var + EPS)

    n_last = N_VPU[-1] * NQ * 32
    qt_s[:, 8:16, :] = jnp.zeros((H // 2, 8, S), i32)
    att_s[A_W:A_W + W_ROWS, :] = bc(jnp.ones((W_ROWS, TQ), f32), i32)
    att_s[A_END - n_last:A_END, :] = bc(jnp.ones((n_last, TQ), f32), i32)
    range_s[...] = jnp.ones(range_s.shape, f32)

    wait("x0")
    cf = c_v[...].astype(f32)
    silu_c = jnp.broadcast_to(cf / (1.0 + jnp.exp(-cf)), (16, D)).astype(bf16)
    r_s[0:16, 0:D] = silu_c.astype(f32)
    zero = lax.shift_right_logical(jnp.sum(jnp.where(cf > 0, 1, 0)), 16)
    xn0 = normed(0, 2 * TK)
    x1_s[0][0:2 * TK, :] = xn0

    def modulation(c0, n):
        return _dot(silu_c, wmod_v[:, c0:c0 + n])[0:8].astype(bf16).astype(f32)

    wait("mod")
    shift = modulation(0, D)[0:1]
    scale = (1.0 + modulation(D, D)).astype(bf16).astype(f32)[0:1]
    h_s[0:TK, :] = bc((xn0 * scale + shift).astype(bf16), i32)

    def hold(ref, row, x):
        ref[_aligned(row + zero * 16, 16, 16), 0:128] = x.astype(ref.dtype)

    side = []

    def release(x, n):
        for i in range(min(n, len(side))):
            r = i * (x.shape[0] // 16) // n * 16
            ref, row, fn, *args = side.pop(0)
            hold(ref, row, x[r:r + 16, 0:128])
            fn(*args)

    def ada_ln(r, n=1):
        h_s[r * 8:(r + n) * 8, :] = bc((normed(r * 16, n * 16) * scale + shift).astype(bf16), i32)

    def k_proj(b, n=0):
        for g in range(D // 128):
            h = bc(h_s[b * TK // 2:(b + 1) * TK // 2, :], bf16)
            k16 = _dot(h, wqkv_v[:, _tile(D // 128 + g)]).astype(bf16)
            release(k16, n)
            k = bc(k16, i32)
            for j in range(4):
                x = pltpu.roll(k, 128 - 32 * j, 1) if j else k
                att_s[pl.ds((g * 4 + j) * K_ROWS + b % 2 * 128, 128), _tile(b // 2)] = x
                for i, blk in enumerate(VPU_BLOCKS):
                    if blk // 16 == b:
                        kf_s[g * 4 + j, i] = x[blk % 16 * 8:blk % 16 * 8 + 8]

    def q_proj(t, n=0):
        q = _dot_nt(bc(wq_s[...], bf16), bc(h_s[t * 64:(t + 1) * 64, :], bf16)) * Q_SCALE
        q16 = q.astype(bf16)
        release(q16, n)
        qs_s[t // 8][pl.ds(t % 8, D, stride=8), :] = q
        for e in range(2):
            qt_s[:, e * 16:e * 16 + 8, _tile(t)] = bc(q16, i32).reshape(H // 2, 16, 128)[:, e * 8:e * 8 + 8]

    def q_regroup(e, hd):
        qf_s[hd, e, :, :, 0:128] = qs_s[e][_tile(hd), :].reshape(DH, 8, 128)

    def w_transpose(src, k, c):
        wt_s[0:D, c:c + 128] = src[k:k + 128, :].T

    def w_operands(dst, i, k0, k1, c0, w):
        blocks = [wt_s[r + i * 16:r + i * 16 + 16, k + c0:k + c0 + w] for r in (0, HD) for k in (k0, k1)]
        for n, x in enumerate(_left_operands(*blocks)):
            dst[n, i * 8:i * 8 + 8, c0:c0 + w] = x

    def gate_up_operands(i):
        blocks = [wgu_v[n, i * 16:i * 16 + 16, c:c + HD] for n in range(2) for c in (0, HD)]
        for n, x in enumerate(_left_operands(*blocks)):
            sg_s[n, i * 8:i * 8 + 8, :] = x

    def gate_up_work(i0, i1):
        return [(wgu_v.at[1], F, gate_up_operands, i) for i in range(i0, i1)]

    def spread_k(pair, u, dst, j, d, state=None):
        src = kf_s[pair, j]
        x = jnp.broadcast_to(src[..., u * DH + d:u * DH + d + 1], src.shape)
        y = bc(x, bf16).astype(f32)
        for g in range(2):
            dst[j, g, d, 8:16, :] = y[..., g * 8:g * 8 + 8, :]
        if state is not None:
            state[W_PACE:W_PACE + 8, _tile(3)] = x

    def probs(u, z=0):
        return att_s.at[_aligned(A_P + u * P_ROWS + z * 8, P_ROWS)]

    wait("wk")
    k_proj(0)
    wait("wq")
    wq_s[...] = bc(wqkv_v[:, 0:D].T, i32)
    k_proj(1)
    q_proj(0)
    q_proj(1)
    wait("x1")
    ada_ln(32, 8)
    side.extend((x_v, S, ada_ln, r) for r in range(40, 80))
    q_proj(2, 10)
    q_proj(3, 8)
    for b in range(2, 4):
        k_proj(b, 3)
        q_proj(b + 2, 5)
    wait("x2")
    ada_ln(80, 4)
    side.extend((x_v, S, ada_ln, r) for r in range(84, S // 16))
    side.extend(gate_up_work(0, G1))
    for b in range(4, S // TK):
        k_proj(b, 3)
        q_proj(b + 2, 5)

    wait("wv")
    to_transpose = ([(wo_v, k, k) for k in range(0, D, 128)]
                    + [(wd_v, k, D + k // 128 % 2 * (FS // 2) + k // 256 * 128) for k in range(0, FS, 128)])
    to_spread = [(u, 1 - u, kb_s[u], slice(0, NV - u), d) for u in range(2) for d in range(DH)]
    to_modulate = []

    def v_proj(t, n, shuffle=True):
        for e in range(2):
            v = _dot_nt(bc(wv_s[_tile(e), :], bf16), bc(h_s[t * 64:(t + 1) * 64, :], bf16))
            att_s[pl.ds(A_V + t // NT * D + e * HD, HD), _tile(t % NT)] = bc(v, i32)
            if to_spread and shuffle:
                kf_s[H // 2, zero] = bc(v[0:8], i32)
                spread_k(*to_spread.pop(0))
            if to_transpose and e and shuffle:
                hold(wd_v, F, v[0:16])
                w_transpose(*to_transpose.pop(0))
            release(v, n)
            if to_modulate:
                i, j = to_modulate.pop(0)
                m = modulation((i + 2) * D + j * 128, 128)[0:1]
                m = jnp.broadcast_to(1.0 + m if i == 2 else m, (128, 128)).astype(bf16)
                col_s[i, _tile(j), :] = m.T.astype(f32)

    wv_s[...] = bc(wqkv_v[:, 2 * D:3 * D].T, i32)
    wdt_s[...] = bc(wd_v[FS:F, :].T, i32)
    k0 = bc(kf_s[0].reshape(NV * 8, 128), bf16)[:, 0:DH]
    for _ in range(4):
        spread_k(*to_spread.pop(0))
    for _ in range(4):
        w_transpose(*to_transpose.pop(0))
    more = gate_up_work(G1, G2) + [(wt_s, D, w_operands, so_s, i, 0, HD, 0, HD) for i in range(NR)]
    for hd in range(1, H):
        side.extend([(qs_s[0], D * 8, q_regroup, 0, hd)] + [more.pop(0) for _ in range(hd % 2)])
    for t in range(10, S // 128):
        q_proj(t, 8)
    for hd in range(1, H):
        side.extend([(qs_s[1], D * 8, q_regroup, 1, hd), more.pop(0)])
    side.extend(more)
    for qb in range(NQ):
        v_proj(qb, 5)
        p = bc(jnp.exp2(_dot(k0, bc(qt_s[0, 0:8, _tile(qb * NT, NT)], bf16))), i32)
        for j in range(NV):
            for t in range(NT):
                probs(0)[pl.ds((j * NQ + qb) * 32 + t // 2 * 16, 16), _tile(1 + t % 2 * 2)] = (
                    p[j * 16:j * 16 + 16, _tile(t)])
    v_proj(4, 5)
    v_proj(5, 5, shuffle=False)
    wait("rest")
    side.extend(gate_up_work(G2, F // 16))
    side.extend((wt_s, D, w_operands, sd_s, i, D, D + FS // 2, *c) for c in ((0, 256), (256, 384)) for i in range(NR))
    to_modulate.extend((i, j) for i in range(4) for j in range(D // 128))
    for _ in range(4):
        fn, *args = side.pop(0)[2:]
        fn(*args)
    for t in range(6, S // 128):
        v_proj(t, 4 if t < 13 else 2)
    assert not (side or to_spread or to_transpose or to_modulate)

    def vpu_probs(hd, keys, dst, g, t):
        k = keys[g // 2, g % 2, :, 8:16, :]
        q = jnp.broadcast_to(qf_s[hd, t // 8, :, t % 8:t % 8 + 1, 0:128], k.shape)
        ks, qs = lax.split(k, [1] * DH), lax.split(q, [1] * DH)
        s = ks[0] * qs[0]
        for kd, qd in zip(ks[1:], qs[1:]):
            s = s + kd * qd
        row = (g // 2 * NQ + t // NT) * 32 + t // 2 % 2 * 16 + g % 2 * 8
        dst[pl.ds(row, 8), _tile(1 + t % 2 * 2)] = bc(jnp.exp2(s.reshape(8, 128)), i32)

    def vpu_block(u, qb, blk):
        rows = pl.ds((VPU_BLOCKS.index(blk) * NQ + qb) * 32, 32)
        x = [bc(probs(u)[rows, _tile(n)], f32) for n in (1, 3)]
        return jnp.concatenate([x[0][:16], x[1][:16], x[0][16:], x[1][16:]], axis=1)

    def pv(hd, c, p):
        return _dot(bc(att_s[_aligned(A_V + c // NT * D + hd * DH, DH), _tile(c % NT)], f32), p)

    def save(hd, qb, l, acc):
        acc_s[hd, :, _aligned(qb * TQ, TQ, TQ)] = acc
        for t in range(NT):
            l_s[qb * NT + t, _aligned(hd * 8, 8), :] = l[:, _tile(t)]

    def finish(hd, qb, l, acc):
        save(hd, qb, l, acc)
        range_s[0] += l + (jnp.abs(acc[:8]) + jnp.abs(acc[8:]))
        range_s[1] = jnp.minimum(range_s[1], l)

    def carried(pair, state):
        c, qb, hd = NC - 1, NQ - 1, pair * 2 + 1
        l = bc(state[W_SUM:W_SUM + 8, :], f32)
        blocks = []
        for b in range(7, -1, -1):
            if c * 8 + b in VPU_BLOCKS:
                p = vpu_block(1, qb, c * 8 + b)
            else:
                p = jnp.exp2(bc(state[pl.ds(W_SCORE + b * 16, 16), :], f32))
            l = (l + p[8:]) + p[:8]
            blocks.insert(0, p)

        def rest():
            acc = pv(hd, c, jnp.concatenate(blocks, axis=0))
            finish(hd, qb, l, acc + bc(state[W_ACC:W_ACC + 16, :], f32))
        return rest

    def attend(pair, carry):
        state = att_s.at[_aligned(A_W + zero * 8, W_ROWS)]
        k_ref = att_s.at[_aligned(pair * K_ROWS, K_ROWS)]
        kb_last = kb_last_s.at[pl.ds(zero, NV)]
        ahead = [jnp.minimum(pair + n, H // 2 - 1) for n in range(3)]
        span = (len(MXU_BLOCKS) + NC) * NQ + (TRAIL - LEAD) / 2
        due = _Agenda()
        for u in range(2):
            hd, dst, last = ahead[u] * 2 + 1 - u, probs(1 - u, zero), NV - u
            due.add([functools.partial(vpu_probs, hd, kb_last if g // 2 >= last else kb_s[u], dst, g, t)
                     for g in range(2 * NV) for t in range(S // 128)], LEAD + u * span, span)
            for n in range(NV * DH):
                j, d = n // DH, DH - 1 - n % DH if n // DH % 2 else n % DH
                frac = (n + DH + 0.1) / (NV * DH)
                if j >= last:
                    due.add([functools.partial(spread_k, ahead[u], 1 - u, kb_last_s, j, d, state)],
                            LEAD + 3, span * (frac - 1))
                else:
                    due.add([functools.partial(spread_k, ahead[u + 1], 1 - u, kb_s[u], j, d, state)],
                            LEAD, span * (u + frac))
        ready, sums, accs = {}, {}, {}

        def stash(row, x, lanes=slice(None)):
            state[pl.ds(row, x.shape[0]), lanes] = bc(x, i32)

        def add_to_sum(key, p):
            l = sums[key] + p[8:] if key in sums else p[8:]
            sums[key] = l + p[:8]

        rest = carried(jnp.maximum(pair - 1, 0), state)
        steps = [(u, qb, c) for u in range(2) for qb in range(NQ) for c in range(NC)]
        for i, (u, qb, c) in enumerate(steps):
            blocks = MXU_BLOCKS[SEGMENT[c]:SEGMENT[c + 1]]
            q = bc(qt_s[pair, u * 8:u * 16 + 8, _tile(qb * NT, NT)], bf16)
            ks, issued = [], []
            for b in blocks:
                due.tick()
                issued.append(due.now)
                ks.append(k_ref[pl.ds(b % 32 * 8, 8), _tile(b // 32)])
            s = _dot(bc(jnp.concatenate(ks, axis=0), bf16)[:, 0:(u + 1) * DH], q)
            due.tick()
            if i == 0:
                rest()
            else:
                up, qp, cp = steps[i - 1]
                o = pv(pair * 2 + up, cp, jnp.concatenate([ready.pop((up, qp, cp, b)) for b in range(8)], axis=0))
                accs[up, qp] = o + accs[up, qp] if cp else o
                if cp == NC - 1:
                    finish(pair * 2 + up, qp, sums[up, qp], accs[up, qp])
            if i + 1 < len(steps):
                for b in range(7, 7 - N_VPU[c], -1):
                    ready[u, qb, c, b] = p = vpu_block(u, qb, c * 8 + b)
                    add_to_sum((u, qb), p)
            for n, b in enumerate(blocks):
                sb = s[n * 16:(n + 1) * 16]
                if (u, qb, b // 8) == steps[-1]:
                    due.add([functools.partial(stash, W_SCORE + b % 8 * 16, sb)], issued[n] - due.now, SCORE_DELAY)
                    continue
                ready[u, qb, b // 8, b % 8] = p = jnp.exp2(sb)
                add_to_sum((u, qb), p)
                t = issued[n] % 2
                due.add([functools.partial(stash, W_PACE, sums[u, qb][:, _tile(2 + t)], _tile(1 + t * 2))],
                        issued[n] - due.now, SUM_DELAY)
        due.flush()
        stash(W_SUM, sums[1, NQ - 1])
        stash(W_ACC, accs[1, NQ - 1])
        return carry

    lax.fori_loop(0, H // 2, attend, 0)
    carried(H // 2 - 1, att_s.at[pl.ds(A_W, W_ROWS)])()

    unsafe = jnp.sum(jnp.where(range_s[0] < SAFE, 0, 1) + jnp.where(range_s[1] > 1.0 / SAFE, 0, 1))

    @pl.when(unsafe > 0)
    def _():
        def with_max(i, carry):
            hd, qb = i // NQ, i % NQ
            k = att_s[_aligned(hd // 2 * K_ROWS, K_ROWS), :]
            k = bc(jnp.concatenate([k[:, _tile(n)] for n in range(NT)], axis=0), bf16)[:, 0:2 * DH]
            s = _dot(k, bc(qt_s[hd // 2, _aligned(hd % 2 * 8, 16), _aligned(qb * TQ, TQ, TQ)], bf16))
            p = jnp.exp2(s - jnp.max(s, axis=0, keepdims=True))
            acc = pv(hd, 0, p[0:CK])
            for c in range(1, NC):
                acc = pv(hd, c, p[c * CK:(c + 1) * CK]) + acc
            save(hd, qb, p.reshape(S // 8, 8, TQ).sum(axis=0), acc)
            return carry

        lax.fori_loop(0, H * NQ, with_max, 0)

    later = _Agenda()

    def held(ref, row, fn, *args):
        def run(y, r):
            hold(ref, row, y[r * 16:r * 16 + 16, 0:128])
            fn(*args)
        return run

    def matmul(lhs, r0, rows, rhs, *done):
        def product(n, acc=None):
            y = _dot(bc(lhs[n, r0 * 8:(r0 + rows) * 8, :], bf16), rhs[n])
            if acc is not None:
                y = y + acc
            for r in range(rows):
                later.tick(y, r)
            return y
        return _strassen(product, *done)

    cells = [(r, t) for t in range(2) for r in range(NR - 1, -1, -1)]
    attn_ops, h_ops, x_t, stat = {}, {}, {}, {}

    def assemble(ops, b):
        return [jnp.concatenate([jnp.concatenate([ops[b, r, t][n] for t in range(2)], axis=1)
                                 for r in range(NR)], axis=0).astype(bf16) for n in range(7)]

    def attn_cell(b, r, t):
        attn_ops[b, r, t] = _right_operands(*[acc_s[hd, :, _tile(c)] * r_s[hd:hd + 1, _tile(c)]
                                              for hd in (r, r + NR) for c in (b * NT + t, b * NT + 2 + t)])

    def transpose_x(b, i, j):
        x_t[b, i, j] = x_v[b * TB + j * HT:b * TB + (j + 1) * HT, i * HD:(i + 1) * HD].T

    def column(n, rows):
        return jnp.concatenate([col_s[n, rows, :]] * 2, axis=1)

    def before_wo(b, span):
        for t in (0, 2, 1, 3):
            t += b * NT
            r_s[:, _tile(t)] = 1.0 / sum(l_s[t, pl.ds(e, H, stride=8), :] for e in range(8))
        for i, j in ((0, 1), (1, 1), (1, 0), (0, 0)):
            if b:
                later.add([held(x_v, S, transpose_x, b, i, j)], 0, span * (2 * i + j) / 4)
            else:
                transpose_x(b, i, j)
        if b:
            later.add([held(acc_s.at[H], 0, attn_cell, b, r, t) for r, t in cells], 0, span)
        else:
            for r, t in cells:
                attn_cell(b, r, t)

    def wo(b):
        def done(i, j, y):
            rows = slice(i * HD, (i + 1) * HD)
            x1 = x_t[b, i, j].astype(f32) + column(0, rows) * y
            x1_s[b][rows, j * HT:(j + 1) * HT] = x1
            for r in range(0, HD, 8):
                stat[b, j] = stat[b, j] + x1[r:r + 8] if (b, j) in stat else x1[r:r + 8]
        matmul(so_s, 0, NR, assemble(attn_ops, b), done)

    def x1_view(b, k):
        return x1_s[b].at[_aligned(zero * 8 * k, D)]

    def centered(k, b, r, t):
        x1 = x1_view(b, k)
        return [x1[pl.ds(i * HD + r * 16, 16), _tile(j * 2 + t)] - stat[b, t, "mean"][j]
                for i in range(2) for j in range(2)]

    def variance_cell(b, r, t):
        if (b, t, "mean") not in stat:
            stat[b, t, "mean"] = [jnp.sum(stat[b, j][:, _tile(t)], axis=0, keepdims=True) * (1.0 / D)
                                  for j in range(2)]
        xc = centered(1, b, r, t)
        for j in range(2):
            s = xc[j] * xc[j] + xc[2 + j] * xc[2 + j]
            s = s[:8] + s[8:]
            stat[b, t, j] = stat[b, t, j] + s if (b, t, j) in stat else s

    def ada_ln_cell(b, r, t):
        if (b, t, "rstd") not in stat:
            stat[b, t, "rstd"] = [lax.rsqrt(jnp.sum(stat[b, t, j], axis=0, keepdims=True) * (1.0 / D) + EPS)
                                  for j in range(2)]
        hs = []
        for n, xc in enumerate(centered(2, b, r, t)):
            rows = pl.ds(n // 2 * HD + r * 16, 16)
            hs.append(xc * stat[b, t, "rstd"][n % 2] * col_s[2, rows, :] + col_s[1, rows, :])
        h_ops[b, r, t] = _right_operands(*hs)

    def after_wo(b, span):
        for fn, f0, f1 in ((variance_cell, 0, 0.35), (ada_ln_cell, 0.37, 0.63)):
            later.add([held(x1_s[b], D, fn, b, r, t) for r, t in cells], span * f0, span * f1)

    def out_copy(b, i):
        rows, cols = pl.ds(b * TB, TB), pl.ds(i * 128, 128)
        return pltpu.make_async_copy(o_v.at[rows, cols], out_h.at[rows, cols], sem.at[len(groups) + b * 2 + i % 2])

    def ffn(b):
        h = assemble(h_ops, b)
        acts = []
        for j in [FS] + list(range(0, FS, 128)):
            g1, g2, u1, u2 = matmul(sg_s, j // 16, min(128, F - j) // 16, h)
            acts.append((_geglu(g1, u1), _geglu(g2, u2)))
            if j == 256 and 0 < b < NB - 1:
                wo(b + 1)
                after_wo(b + 1, 385)
        y0 = _dot(bc(wdt_s[...], bf16), jnp.concatenate(acts.pop(0), axis=1).astype(bf16))
        act = [x.astype(bf16) for x in _right_operands(
            *[jnp.concatenate([x[j] for x in acts[i::2]], axis=0) for i in range(2) for j in range(2)])]
        for e in range(2):
            def done(i, j, y):
                rows, cols = _tile(2 * i + e), slice(j * HT, (j + 1) * HT)
                o_v[b * TB + j * HT:b * TB + (j + 1) * HT, rows] = (
                    x1_view(b, 3)[rows, cols] + column(3, rows) * (y + y0[rows, cols])).astype(bf16).T

            def send(*_, e=e):
                for i in range(2):
                    out_copy(b, 2 * i + e).start()
                hold(o_v, S, jnp.zeros((16, 128), bf16))
                next_lhs = sg_s if b + 1 < NB else sd_s
                next_lhs[7, _aligned(zero * 8, 8), 0:128] = bc(o_v[S:S + 16, 0:128], i32)
            matmul(sd_s, e * 8, 8, act, done)
            later.add([send], 120 if b + 1 < NB else 24, 0)

    before_wo(0, 0)
    before_wo(1, 60)
    wo(0)
    after_wo(0, 98)
    wo(1)
    after_wo(1, 590)
    for b in range(NB):
        if 0 < b < NB - 1:
            before_wo(b + 1, 176)
        ffn(b)
    later.flush()
    for b in range(NB):
        for i in range(4):
            out_copy(b, i).wait()


def _scratch_shapes():
    v = pltpu.VMEM
    return [
        v((A_END + 8, TQ), i32),
        [v((NV, 2, DH, 16, 128), f32)] * 2,
        v((NV + 1, 2, DH, 16, 128), f32),
        v((H // 2, 24, S), i32),
        v((H, 2, DH, 8, 256), f32),
        [v((D * 8 + 32, 128), f32)] * 2,
        v((H // 2 + 1, NV, 8, 128), i32),
        v((H + 2, DH, S), f32),
        v((S // 128, H * 8 + 8, 128), f32),
        v((H, S), f32),
        v((2, 8, TQ), f32),
        v((S // 2, D), i32),
        v((D // 2, D), i32),
        v((D // 2, D), i32),
        v((7, HD // 2, HD), i32),
        v((8, F // 2, HD), i32),
        v((8, HD // 2, FS // 2), i32),
        [v((D + 32, TB), f32)] * NB,
        v((S + 32, D), bf16),
        v((D, 3 * D), bf16),
        v((D, D), bf16),
        v((2, F + 32, D), bf16),
        v((F + 32, D), bf16),
        v((D, 6 * D), bf16),
        v((S + 32, D), bf16),
        v((4, D, 128), f32),
        v((D + 32, D + FS), bf16),
        v((D // 2, F - FS), i32),
        v((1, D), bf16),
        pltpu.SemaphoreType.DMA((8 + 2 * NB,)),
    ]


@jax.jit
def pallas_adaLN_cond__mha_block__geglu_ffn__prompt_kernel(
    A_x: jax.Array,
    A_wqkv: jax.Array,
    A_wo: jax.Array,
    B_x: jax.Array,
    B_w_gate: jax.Array,
    B_w_up: jax.Array,
    B_w_down: jax.Array,
    c: jax.Array,
    w_mod: jax.Array,
):
    del B_x
    hbm = pl.BlockSpec(memory_space=pltpu.HBM)
    out = pl.pallas_call(
        _kernel,
        out_shape=jax.ShapeDtypeStruct((S, D), bf16),
        in_specs=[hbm] * 8,
        out_specs=hbm,
        scratch_shapes=_scratch_shapes(),
        compiler_params=pltpu.CompilerParams(vmem_limit_bytes=115 * 1024 * 1024),
    )(A_x.reshape(S, D), A_wqkv, A_wo, B_w_gate.T, B_w_up.T, B_w_down, c, w_mod)
    return out.reshape(1, S, D)
```

```python
import functools

import jax
import jax.numpy as jnp
import numpy as np
from jax import lax
from jax.experimental import pallas as pl
from jax.experimental.pallas import tpu as pltpu

S, D, H, DH, F = 2048, 512, 32, 16, 1376
EPS = 1e-5
Q_SCALE = DH ** -0.5 * float(np.log2(np.e))
SAFE_LOW, SAFE_HIGH = 2.0 ** -60, 2.0 ** 120
f32, bf16, i32 = jnp.float32, jnp.bfloat16, jnp.int32
bc = pltpu.bitcast

TQ, CK = 512, 128
NQ, NC, NT = S // TQ, S // CK, TQ // 128
N_VPU = [2, 1, 1, 1, 1, 2, 1, 2, 1, 1, 2, 1, 1, 1, 1, 1]
VPU_BLOCKS = [c * 8 + b for c in range(NC) for b in range(8 - N_VPU[c], 8)]
MXU_BLOCKS = [c * 8 + b for c in range(NC) for b in range(7 - N_VPU[c], -1, -1)]
NV = len(VPU_BLOCKS)
SEGMENT = [int(n) for n in np.cumsum([0, 8, 6, 7, 7, 7, 7, 6, 7, 6, 7, 7, 7, 6, 7, 7, 6])]
LEAD, TRAIL, SUM_DELAY, SCORE_DELAY = 6.28, 2.55, 11, 9

K_ROWS, P_ROWS = S // 8, NV * NQ * 32
W_PACE, W_ACC, W_SUM, W_SCORE, W_ROWS = 0, 8, 24, 32, 160
A_V = H // 2 * K_ROWS
A_W = A_V + NQ * D
A_P = A_W + W_ROWS
A_END = A_P + 2 * P_ROWS

TK = 256
TB = 512
NB = S // TB
HD, HT = D // 2, TB // 2
NR = HD // 16
FS = 1280
G1, G2 = 24, 56


def _dot(a, b):
    return jnp.dot(a, b, preferred_element_type=f32)


def _dot_nt(a, b):
    return lax.dot_general(a, b, (((1,), (1,)), ((), ())), preferred_element_type=f32)


def _aligned(start, size, multiple=8):
    return pl.ds(start if isinstance(start, int) else pl.multiple_of(start, multiple), size)


def _tile(i, n=1):
    return slice(i * 128, (i + n) * 128)


def _left_operands(a11, a12, a21, a22):
    f = [x.astype(f32) for x in (a11, a12, a21, a22)]
    ops = [(f[0] + f[3]).astype(bf16), (f[2] + f[3]).astype(bf16), a11, a22,
           (f[0] + f[1]).astype(bf16), (f[2] - f[0]).astype(bf16), (f[1] - f[3]).astype(bf16)]
    return [bc(x, i32) for x in ops]


def _right_operands(b11, b12, b21, b22):
    return [b11 + b22, b11, b12 - b22, b21 - b11, b22, b11 + b12, b21 + b22]


def _strassen(product, done=lambda i, j, c: c):
    m1 = product(0)
    m2 = product(1)
    c22 = m1 - m2
    m3 = product(2)
    c22 = c22 + m3
    m5 = product(4)
    c12 = done(0, 1, m3 + m5)
    c11 = m1 - m5
    c22 = done(1, 1, product(5, c22))
    m4 = product(3)
    c21 = done(1, 0, m2 + m4)
    c11 = c11 + m4
    c11 = done(0, 0, product(6, c11))
    return c11, c12, c21, c22


def _geglu(g, up):
    k = float(np.sqrt(2.0 / np.pi))
    th = jnp.tanh(g * (k + (k * 0.044715) * (g * g)))
    hg = 0.5 * g
    return (hg + hg * th) * up


class _Agenda:
    def __init__(self):
        self.now, self.todo = 0, []

    def add(self, fns, start, span):
        for k, fn in enumerate(fns):
            self.todo.append((self.now + start + span * (k + 1) / len(fns), fn))
        self.todo.sort(key=lambda w: w[0])

    def tick(self, *args):
        self.now += 1
        while self.todo and self.todo[0][0] <= self.now:
            self.todo.pop(0)[1](*args)

    def flush(self):
        while self.todo:
            self.todo.pop(0)[1]()


def _kernel(x_h, wqkv_h, wo_h, wgt_h, wut_h, wd_h, c_h, wmod_h, out_h,
            att_s, kb_s, kb_last_s, qt_s, qf_s, qs_s, kf_s, acc_s, l_s, r_s, range_s,
            h_s, wq_s, wv_s, so_s, sg_s, sd_s, x1_s,
            x_v, wqkv_v, wo_v, wgu_v, wd_v, wmod_v, o_v, col_s, wt_s, wdt_s, v0_s, c_v, sem):
    groups = {}

    def start(name, src, dst):
        group = groups.setdefault(name, [])
        group.append(pltpu.make_async_copy(src, dst, sem.at[list(groups).index(name)]))
        group[-1].start()

    def wait(name):
        for copy in groups[name]:
            copy.wait()

    def start_gate_up(name, i0, i1):
        rows = pl.ds(i0 * 16, (i1 - i0) * 16)
        start(name, wgt_h.at[rows], wgu_v.at[0, rows])
        start(name, wut_h.at[rows], wgu_v.at[1, rows])

    start("x0", c_h, c_v)
    start("x0", x_h.at[pl.ds(0, 2 * TK)], x_v.at[pl.ds(0, 2 * TK)])
    start("mod", wmod_h.at[:, pl.ds(0, 2 * D)], wmod_v.at[:, pl.ds(0, 2 * D)])
    start("wk", wqkv_h.at[:, pl.ds(D, D)], wqkv_v.at[:, pl.ds(D, D)])
    start("wq", wqkv_h.at[:, pl.ds(0, D)], wqkv_v.at[:, pl.ds(0, D)])
    start("x1", x_h.at[pl.ds(2 * TK, 3 * TK)], x_v.at[pl.ds(2 * TK, 3 * TK)])
    start("x2", x_h.at[pl.ds(5 * TK, 3 * TK)], x_v.at[pl.ds(5 * TK, 3 * TK)])
    start_gate_up("x2", 0, G1)
    start("wv", wqkv_h.at[:, pl.ds(2 * D, D)], wqkv_v.at[:, pl.ds(2 * D, D)])
    start("wv", wo_h, wo_v)
    start("wv", wd_h, wd_v.at[pl.ds(0, F)])
    start_gate_up("wv", G1, G2)
    start_gate_up("rest", G2, F // 16)
    start("rest", wmod_h.at[:, pl.ds(2 * D, 4 * D)], wmod_v.at[:, pl.ds(2 * D, 4 * D)])

    def normed(r0, n):
        x = x_v[r0:r0 + n, :].astype(f32)
        xc = x - jnp.sum(x, axis=1, keepdims=True) * (1.0 / D)
        var = jnp.sum(xc * xc, axis=1, keepdims=True) * (1.0 / D)
        return xc * lax.rsqrt(var + EPS)

    n_last = N_VPU[-1] * NQ * 32
    qt_s[:, 8:16, :] = jnp.zeros((H // 2, 8, S), i32)
    att_s[A_W:A_W + W_ROWS, :] = bc(jnp.ones((W_ROWS, TQ), f32), i32)
    att_s[A_P:A_P + P_ROWS, _tile(1)] = att_s[A_P:A_P + P_ROWS, _tile(3)] = jnp.zeros((P_ROWS, 128), i32)
    att_s[A_END - n_last:A_END, :] = bc(jnp.ones((n_last, TQ), f32), i32)
    range_s[...] = jnp.ones(range_s.shape, f32)

    wait("x0")
    cf = c_v[...].astype(f32)
    silu_c = jnp.broadcast_to(cf / (1.0 + jnp.exp(-cf)), (16, D)).astype(bf16)
    r_s[0:16, 0:D] = silu_c.astype(f32)
    zero = lax.shift_right_logical(jnp.sum(jnp.where(cf > 0, 1, 0)), 16)
    xn0 = normed(0, 2 * TK)
    x1_s[0][0:2 * TK, :] = xn0

    def modulation(c0, n):
        return _dot(silu_c, wmod_v[:, c0:c0 + n])[0:8].astype(bf16).astype(f32)

    wait("mod")
    shift = modulation(0, D)[0:1]
    scale = (1.0 + modulation(D, D)).astype(bf16).astype(f32)[0:1]
    h_s[0:TK, :] = bc((xn0 * scale + shift).astype(bf16), i32)

    def hold(ref, row, x):
        ref[_aligned(row + zero * 16, 16, 16), 0:128] = x.astype(ref.dtype)

    side = []

    def release(x, n):
        for i in range(min(n, len(side))):
            r = i * (x.shape[0] // 16) // n * 16
            ref, row, fn, *args = side.pop(0)
            hold(ref, row, x[r:r + 16, 0:128])
            fn(*args)

    def ada_ln(r, n=1):
        h_s[r * 8:(r + n) * 8, :] = bc((normed(r * 16, n * 16) * scale + shift).astype(bf16), i32)

    def k_proj(b, n=0):
        for g in range(D // 128):
            h = bc(h_s[b * TK // 2:(b + 1) * TK // 2, :], bf16)
            k16 = _dot(h, wqkv_v[:, _tile(D // 128 + g)]).astype(bf16)
            release(k16, n)
            k = bc(k16, i32)
            for j in range(4):
                x = pltpu.roll(k, 128 - 32 * j, 1) if j else k
                att_s[pl.ds((g * 4 + j) * K_ROWS + b % 2 * 128, 128), _tile(b // 2)] = x
                for i, blk in enumerate(VPU_BLOCKS):
                    if blk // 16 == b:
                        kf_s[g * 4 + j, i] = x[blk % 16 * 8:blk % 16 * 8 + 8]

    def q_proj(t, n=0):
        q = _dot_nt(bc(wq_s[...], bf16), bc(h_s[t * 64:(t + 1) * 64, :], bf16)) * Q_SCALE
        q16 = q.astype(bf16)
        release(q16, n)
        qs_s[t // 8][pl.ds(t % 8, D, stride=8), :] = q
        for e in range(2):
            qt_s[:, e * 16:e * 16 + 8, _tile(t)] = bc(q16, i32).reshape(H // 2, 16, 128)[:, e * 8:e * 8 + 8]

    def q_regroup(e, hd):
        qf_s[hd, e, :, :, 0:128] = qs_s[e][_tile(hd), :].reshape(DH, 8, 128)

    def w_transpose(src, k, c):
        wt_s[0:D, c:c + 128] = src[k:k + 128, :].T

    def w_operands(dst, i, k0, k1, c0, w):
        blocks = [wt_s[r + i * 16:r + i * 16 + 16, k + c0:k + c0 + w] for r in (0, HD) for k in (k0, k1)]
        for n, x in enumerate(_left_operands(*blocks)):
            dst[n, i * 8:i * 8 + 8, c0:c0 + w] = x

    def gate_up_operands(i):
        blocks = [wgu_v[n, i * 16:i * 16 + 16, c:c + HD] for n in range(2) for c in (0, HD)]
        for n, x in enumerate(_left_operands(*blocks)):
            sg_s[n, i * 8:i * 8 + 8, :] = x

    def gate_up_work(i0, i1):
        return [(wgu_v.at[1], F, gate_up_operands, i) for i in range(i0, i1)]

    def spread_k(pair, u, dst, j, d, state=None):
        src = kf_s[pair, j]
        x = jnp.broadcast_to(src[..., u * DH + d:u * DH + d + 1], src.shape)
        y = bc(x, bf16).astype(f32)
        for g in range(2):
            dst[j, g, d, 8:16, :] = y[..., g * 8:g * 8 + 8, :]
        if state is not None:
            state[W_PACE:W_PACE + 8, _tile(3)] = x

    def probs(u, z=0):
        return att_s.at[_aligned(A_P + u * P_ROWS + z * 8, P_ROWS)]

    wait("wk")
    k_proj(0)
    wait("wq")
    wq_s[...] = bc(wqkv_v[:, 0:D].T, i32)
    k_proj(1)
    q_proj(0)
    q_proj(1)
    wait("x1")
    ada_ln(32, 8)
    side.extend((x_v, S, ada_ln, r) for r in range(40, 80))
    q_proj(2, 10)
    q_proj(3, 8)
    for b in range(2, 4):
        k_proj(b, 3)
        q_proj(b + 2, 5)
    wait("x2")
    ada_ln(80, 4)
    side.extend((x_v, S, ada_ln, r) for r in range(84, S // 16))
    side.extend(gate_up_work(0, G1))
    for b in range(4, S // TK):
        k_proj(b, 3)
        q_proj(b + 2, 5)

    wait("wv")
    to_transpose = ([(wo_v, k, k) for k in range(0, D, 128)]
                    + [(wd_v, k, D + k // 128 % 2 * (FS // 2) + k // 256 * 128) for k in range(0, FS, 128)])
    to_spread = [(u, 1 - u, kb_s[u], slice(0, NV - u), d) for u in range(2) for d in range(DH)]
    to_modulate = []

    def v_proj(t, n, shuffle=True):
        for e in range(2):
            v = _dot_nt(bc(wv_s[_tile(e), :], bf16), bc(h_s[t * 64:(t + 1) * 64, :], bf16))
            att_s[pl.ds(A_V + t // NT * D + e * HD, HD), _tile(t % NT)] = bc(v, i32)
            if to_spread and shuffle:
                kf_s[H // 2, zero] = bc(v[0:8], i32)
                spread_k(*to_spread.pop(0))
            if to_transpose and e and shuffle:
                hold(wd_v, F, v[0:16])
                w_transpose(*to_transpose.pop(0))
            release(v, n)
            if to_modulate:
                i, j = to_modulate.pop(0)
                m = modulation((i + 2) * D + j * 128, 128)[0:1]
                m = jnp.broadcast_to(1.0 + m if i == 2 else m, (128, 128)).astype(bf16)
                col_s[i, _tile(j), :] = m.T.astype(f32)

    wv_s[...] = bc(wqkv_v[:, 2 * D:3 * D].T, i32)
    wdt_s[...] = bc(wd_v[FS:F, :].T, i32)
    for _ in range(4):
        spread_k(*to_spread.pop(0))
    for _ in range(4):
        w_transpose(*to_transpose.pop(0))
    more = gate_up_work(G1, G2) + [(wt_s, D, w_operands, so_s, i, 0, HD, 0, HD) for i in range(NR)]
    for hd in range(H):
        side.extend([(qs_s[0], D * 8, q_regroup, 0, hd)] + [more.pop(0) for _ in range(hd % 2)])
    for t in range(10, S // 128):
        q_proj(t, 9)
    for hd in range(H):
        side.extend([(qs_s[1], D * 8, q_regroup, 1, hd), more.pop(0)])
    side.extend(more)
    for t in range(7):
        v_proj(t, 5, shuffle=t < 6)
    wait("rest")
    side.extend(gate_up_work(G2, F // 16))
    side.extend((wt_s, D, w_operands, sd_s, i, D, D + FS // 2, *c) for c in ((0, 256), (256, 384)) for i in range(NR))
    to_modulate.extend((i, j) for i in range(4) for j in range(D // 128))
    for _ in range(4):
        fn, *args = side.pop(0)[2:]
        fn(*args)
    for t in range(7, S // 128):
        v_proj(t, 3 if t < 9 else 4)
    v0_s[...] = jnp.concatenate(
        [bc(att_s[pl.ds(A_V + blk // 32 * D, DH), pl.ds(blk % 32 * 16, 16)], f32) for blk in VPU_BLOCKS],
        axis=1).astype(bf16)
    assert not (side or to_spread or to_transpose or to_modulate)

    def vpu_probs(hd, keys, dst, g, t):
        k = keys[g // 2, g % 2, :, 8:16, :]
        q = jnp.broadcast_to(qf_s[hd, t // 8, :, t % 8:t % 8 + 1, 0:128], k.shape)
        ks, qs = lax.split(k, [1] * DH), lax.split(q, [1] * DH)
        s = ks[0] * qs[0]
        for kd, qd in zip(ks[1:], qs[1:]):
            s = s + kd * qd
        row = (g // 2 * NQ + t // NT) * 32 + t // 2 % 2 * 16 + g % 2 * 8
        dst[pl.ds(row, 8), _tile(1 + t % 2 * 2)] = bc(jnp.exp2(s.reshape(8, 128)), i32)

    def vpu_block(u, qb, blk):
        rows = pl.ds((VPU_BLOCKS.index(blk) * NQ + qb) * 32, 32)
        x = [bc(probs(u)[rows, _tile(n)], f32) for n in (1, 3)]
        return jnp.concatenate([x[0][:16], x[1][:16], x[0][16:], x[1][16:]], axis=1)

    def pv(hd, c, p):
        return _dot(bc(att_s[_aligned(A_V + c // NT * D + hd * DH, DH), _tile(c % NT)], f32), p)

    def save(hd, qb, l, acc):
        acc_s[hd, :, _aligned(qb * TQ, TQ, TQ)] = acc
        for t in range(NT):
            l_s[qb * NT + t, _aligned(hd * 8, 8), :] = l[:, _tile(t)]

    def finish(hd, qb, l, acc):
        save(hd, qb, l, acc)
        range_s[0] += l + (jnp.abs(acc[:8]) + jnp.abs(acc[8:]))
        range_s[1] = jnp.minimum(range_s[1], l)

    def carried(pair, state):
        c, qb, hd = NC - 1, NQ - 1, pair * 2 + 1
        l = bc(state[W_SUM:W_SUM + 8, :], f32)
        blocks = []
        for b in range(7, -1, -1):
            if c * 8 + b in VPU_BLOCKS:
                p = vpu_block(1, qb, c * 8 + b)
            else:
                p = jnp.exp2(bc(state[pl.ds(W_SCORE + b * 16, 16), :], f32))
            l = (l + p[8:]) + p[:8]
            blocks.insert(0, p)

        def rest():
            acc = pv(hd, c, jnp.concatenate(blocks, axis=0))
            finish(hd, qb, l, acc + bc(state[W_ACC:W_ACC + 16, :], f32))
        return rest

    def attend(pair, carry):
        state = att_s.at[_aligned(A_W + zero * 8, W_ROWS)]
        k_ref = att_s.at[_aligned(pair * K_ROWS, K_ROWS)]
        kb_last = kb_last_s.at[pl.ds(zero, NV)]
        ahead = [(pair + n) & (H // 2 - 1) for n in range(3)]
        span = (len(MXU_BLOCKS) + NC) * NQ + (TRAIL - LEAD) / 2
        due = _Agenda()
        for u in range(2):
            hd, dst, last = ahead[u] * 2 + 1 - u, probs(1 - u, zero), NV - u
            due.add([functools.partial(vpu_probs, hd, kb_last if g // 2 >= last else kb_s[u], dst, g, t)
                     for g in range(2 * NV) for t in range(S // 128)[::-1 if g % 2 else 1]], LEAD + u * span, span)
            for n in range(NV * DH):
                j, d = n // DH, DH - 1 - n % DH if n // DH % 2 else n % DH
                frac = (n + DH + 0.35) / (NV * DH)
                if j >= last:
                    due.add([functools.partial(spread_k, ahead[u], 1 - u, kb_last_s, j, d, state)],
                            LEAD + 3, span * (frac - 1))
                else:
                    due.add([functools.partial(spread_k, ahead[u + 1], 1 - u, kb_s[u], j, d, state)],
                            LEAD, span * (u + frac))
        ready, sums, accs = {}, {}, {}

        def stash(row, x, lanes=slice(None)):
            state[pl.ds(row, x.shape[0]), lanes] = bc(x, i32)

        def add_to_sum(key, p):
            l = sums[key] + p[8:] if key in sums else p[8:]
            sums[key] = l + p[:8]

        rest = carried(jnp.maximum(pair - 1, 0), state)
        steps = [(u, qb, c) for u in range(2) for qb in range(NQ) for c in range(NC)]
        for i, (u, qb, c) in enumerate(steps):
            blocks = MXU_BLOCKS[SEGMENT[c]:SEGMENT[c + 1]]
            q = bc(qt_s[pair, u * 8:u * 16 + 8, _tile(qb * NT, NT)], bf16)
            ks, issued = [], []
            for b in blocks:
                due.tick()
                issued.append(due.now)
                ks.append(k_ref[pl.ds(b % 32 * 8, 8), _tile(b // 32)])
            s = _dot(bc(jnp.concatenate(ks, axis=0), bf16)[:, 0:(u + 1) * DH], q)
            due.tick()
            if i == 0:
                rest()
            else:
                up, qp, cp = steps[i - 1]
                o = pv(pair * 2 + up, cp, jnp.concatenate([ready.pop((up, qp, cp, b)) for b in range(8)], axis=0))
                accs[up, qp] = o + accs[up, qp] if cp else o
                if cp == NC - 1:
                    finish(pair * 2 + up, qp, sums[up, qp], accs[up, qp])
            if i + 1 < len(steps):
                for b in range(7, 7 - N_VPU[c], -1):
                    ready[u, qb, c, b] = p = vpu_block(u, qb, c * 8 + b)
                    add_to_sum((u, qb), p)
            for n, b in enumerate(blocks):
                sb = s[n * 16:(n + 1) * 16]
                if (u, qb, b // 8) == steps[-1]:
                    due.add([functools.partial(stash, W_SCORE + b % 8 * 16, sb)], issued[n] - due.now, SCORE_DELAY)
                    continue
                ready[u, qb, b // 8, b % 8] = p = jnp.exp2(sb)
                add_to_sum((u, qb), p)
                t = 1 - issued[n] % 2
                due.add([functools.partial(stash, W_PACE, sums[u, qb][:, _tile(2 + t)], _tile(1 + t * 2))],
                        issued[n] - due.now, SUM_DELAY)
        due.flush()
        stash(W_SUM, sums[1, NQ - 1])
        stash(W_ACC, accs[1, NQ - 1])
        return carry

    lax.fori_loop(0, H // 2, attend, 0)
    carried(H // 2 - 1, att_s.at[pl.ds(A_W, W_ROWS)])()
    for qb in range(NQ):
        p = jnp.concatenate([vpu_block(0, qb, blk) for blk in VPU_BLOCKS], axis=0)
        l = jnp.concatenate([l_s[qb * NT + t, 0:8, :] for t in range(NT)], axis=1)
        finish(0, qb, l + p.reshape(2 * NV, 8, TQ).sum(axis=0),
               acc_s[0, :, _tile(qb * NT, NT)] + _dot(v0_s[...], p.astype(bf16)))

    unsafe = jnp.sum(jnp.where(range_s[0] < SAFE_HIGH, 0, 1) + jnp.where(range_s[1] > SAFE_LOW, 0, 1))

    @pl.when(unsafe > 0)
    def _():
        def with_max(i, carry):
            hd, qb = i // NQ, i % NQ
            k = att_s[_aligned(hd // 2 * K_ROWS, K_ROWS), :]
            k = bc(jnp.concatenate([k[:, _tile(n)] for n in range(NT)], axis=0), bf16)[:, 0:2 * DH]
            s = _dot(k, bc(qt_s[hd // 2, _aligned(hd % 2 * 8, 16), _aligned(qb * TQ, TQ, TQ)], bf16))
            p = jnp.exp2(s - jnp.max(s, axis=0, keepdims=True))
            acc = pv(hd, 0, p[0:CK])
            for c in range(1, NC):
                acc = pv(hd, c, p[c * CK:(c + 1) * CK]) + acc
            save(hd, qb, p.reshape(S // 8, 8, TQ).sum(axis=0), acc)
            return carry

        lax.fori_loop(0, H * NQ, with_max, 0)

    later = _Agenda()

    def held(ref, row, fn, *args):
        def run(y, r):
            hold(ref, row, y[r * 16:r * 16 + 16, 0:128])
            fn(*args)
        return run

    def matmul(lhs, r0, rows, rhs, *done):
        def product(n, acc=None):
            y = _dot(bc(lhs[n, r0 * 8:(r0 + rows) * 8, :], bf16), rhs[n])
            if acc is not None:
                y = y + acc
            for r in range(rows):
                later.tick(y, r)
            return y
        return _strassen(product, *done)

    cells = [(r, t) for t in range(2) for r in range(NR - 1, -1, -1)]
    attn_ops, h_ops, x_t, stat = {}, {}, {}, {}

    def assemble(ops, b):
        return [jnp.concatenate([jnp.concatenate([ops[b, r, t][n] for t in range(2)], axis=1)
                                 for r in range(NR)], axis=0).astype(bf16) for n in range(7)]

    def attn_cell(b, r, t):
        attn_ops[b, r, t] = _right_operands(*[acc_s[hd, :, _tile(c)] * r_s[hd:hd + 1, _tile(c)]
                                              for hd in (r, r + NR) for c in (b * NT + t, b * NT + 2 + t)])

    def transpose_x(b, i, j):
        x_t[b, i, j] = x_v[b * TB + j * HT:b * TB + (j + 1) * HT, i * HD:(i + 1) * HD].T

    def column(n, rows):
        return jnp.concatenate([col_s[n, rows, :]] * 2, axis=1)

    def before_wo(b, span):
        for t in (0, 2, 1, 3):
            t += b * NT
            r_s[:, _tile(t)] = 1.0 / sum(l_s[t, pl.ds(e, H, stride=8), :] for e in range(8))
        for i, j in ((0, 1), (1, 1), (1, 0), (0, 0)):
            if b:
                later.add([held(x_v, S, transpose_x, b, i, j)], 0, span * (2 * i + j) / 4)
            else:
                transpose_x(b, i, j)
        if b:
            later.add([held(acc_s.at[H], 0, attn_cell, b, r, t) for r, t in cells], 0, span)
        else:
            for r, t in cells:
                attn_cell(b, r, t)

    def wo(b):
        def done(i, j, y):
            rows = slice(i * HD, (i + 1) * HD)
            x1 = x_t[b, i, j].astype(f32) + column(0, rows) * y
            x1_s[b][rows, j * HT:(j + 1) * HT] = x1
            for r in range(0, HD, 8):
                stat[b, j] = stat[b, j] + x1[r:r + 8] if (b, j) in stat else x1[r:r + 8]
        matmul(so_s, 0, NR, assemble(attn_ops, b), done)

    def x1_view(b, k):
        return x1_s[b].at[_aligned(zero * 8 * k, D)]

    def centered(k, b, r, t):
        x1 = x1_view(b, k)
        return [x1[pl.ds(i * HD + r * 16, 16), _tile(j * 2 + t)] - stat[b, t, "mean"][j]
                for i in range(2) for j in range(2)]

    def variance_cell(b, r, t):
        if (b, t, "mean") not in stat:
            stat[b, t, "mean"] = [jnp.sum(stat[b, j][:, _tile(t)], axis=0, keepdims=True) * (1.0 / D)
                                  for j in range(2)]
        xc = centered(1, b, r, t)
        for j in range(2):
            s = xc[j] * xc[j] + xc[2 + j] * xc[2 + j]
            s = s[:8] + s[8:]
            stat[b, t, j] = stat[b, t, j] + s if (b, t, j) in stat else s

    def ada_ln_cell(b, r, t):
        if (b, t, "rstd") not in stat:
            stat[b, t, "rstd"] = [lax.rsqrt(jnp.sum(stat[b, t, j], axis=0, keepdims=True) * (1.0 / D) + EPS)
                                  for j in range(2)]
        hs = []
        for n, xc in enumerate(centered(2, b, r, t)):
            rows = pl.ds(n // 2 * HD + r * 16, 16)
            hs.append(xc * stat[b, t, "rstd"][n % 2] * col_s[2, rows, :] + col_s[1, rows, :])
        h_ops[b, r, t] = _right_operands(*hs)

    def after_wo(b, span):
        for fn, f0, f1 in ((variance_cell, 0, 0.35), (ada_ln_cell, 0.37, 0.63)):
            later.add([held(x1_s[b], D, fn, b, r, t) for r, t in cells], span * f0, span * f1)

    def out_copy(b, i):
        rows, cols = pl.ds(b * TB, TB), pl.ds(i * 128, 128)
        return pltpu.make_async_copy(o_v.at[rows, cols], out_h.at[rows, cols], sem.at[len(groups) + b * 2 + i % 2])

    def ffn(b):
        h = assemble(h_ops, b)
        acts = []
        for j in [FS] + list(range(0, FS, 128)):
            g1, g2, u1, u2 = matmul(sg_s, j // 16, min(128, F - j) // 16, h)
            acts.append((_geglu(g1, u1), _geglu(g2, u2)))
            if j == 256 and 0 < b < NB - 1:
                wo(b + 1)
                after_wo(b + 1, 385)
        y0 = _dot(bc(wdt_s[...], bf16), jnp.concatenate(acts.pop(0), axis=1).astype(bf16))
        act = [x.astype(bf16) for x in _right_operands(
            *[jnp.concatenate([x[j] for x in acts[i::2]], axis=0) for i in range(2) for j in range(2)])]
        for e in range(2):
            def done(i, j, y):
                rows, cols = _tile(2 * i + e), slice(j * HT, (j + 1) * HT)
                o_v[b * TB + j * HT:b * TB + (j + 1) * HT, rows] = (
                    x1_view(b, 3)[rows, cols] + column(3, rows) * (y + y0[rows, cols])).astype(bf16).T

            def send(*_, e=e):
                for i in range(2):
                    out_copy(b, 2 * i + e).start()
                hold(o_v, S, jnp.zeros((16, 128), bf16))
                next_lhs = sg_s if b + 1 < NB else sd_s
                next_lhs[7, _aligned(zero * 8, 8), 0:128] = bc(o_v[S:S + 16, 0:128], i32)
            matmul(sd_s, e * 8, 8, act, done)
            later.add([send], 120 if b + 1 < NB else 24, 0)

    before_wo(0, 0)
    before_wo(1, 45)
    wo(0)
    after_wo(0, 102)
    wo(1)
    after_wo(1, 590)
    for b in range(NB):
        if 0 < b < NB - 1:
            before_wo(b + 1, 176)
        ffn(b)
    later.flush()
    for b in range(NB):
        for i in range(4):
            out_copy(b, i).wait()


def _scratch_shapes():
    v = pltpu.VMEM
    return [
        v((A_END + 8, TQ), i32),
        [v((NV, 2, DH, 16, 128), f32)] * 2,
        v((NV + 1, 2, DH, 16, 128), f32),
        v((H // 2, 24, S), i32),
        v((H, 2, DH, 8, 256), f32),
        [v((D * 8 + 32, 128), f32)] * 2,
        v((H // 2 + 1, NV, 8, 128), i32),
        v((H + 2, DH, S), f32),
        v((S // 128, H * 8 + 8, 128), f32),
        v((H, S), f32),
        v((2, 8, TQ), f32),
        v((S // 2, D), i32),
        v((D // 2, D), i32),
        v((D // 2, D), i32),
        v((7, HD // 2, HD), i32),
        v((8, F // 2, HD), i32),
        v((8, HD // 2, FS // 2), i32),
        [v((D + 32, TB), f32)] * NB,
        v((S + 32, D), bf16),
        v((D, 3 * D), bf16),
        v((D, D), bf16),
        v((2, F + 32, D), bf16),
        v((F + 32, D), bf16),
        v((D, 6 * D), bf16),
        v((S + 32, D), bf16),
        v((4, D, 128), f32),
        v((D + 32, D + FS), bf16),
        v((D // 2, F - FS), i32),
        v((DH, NV * 16), bf16),
        v((1, D), bf16),
        pltpu.SemaphoreType.DMA((8 + 2 * NB,)),
    ]


@jax.jit
def pallas_adaLN_cond__mha_block__geglu_ffn__prompt_kernel(
    A_x: jax.Array,
    A_wqkv: jax.Array,
    A_wo: jax.Array,
    B_x: jax.Array,
    B_w_gate: jax.Array,
    B_w_up: jax.Array,
    B_w_down: jax.Array,
    c: jax.Array,
    w_mod: jax.Array,
):
    del B_x
    hbm = pl.BlockSpec(memory_space=pltpu.HBM)
    out = pl.pallas_call(
        _kernel,
        out_shape=jax.ShapeDtypeStruct((S, D), bf16),
        in_specs=[hbm] * 8,
        out_specs=hbm,
        scratch_shapes=_scratch_shapes(),
        compiler_params=pltpu.CompilerParams(vmem_limit_bytes=115 * 1024 * 1024),
    )(A_x.reshape(S, D), A_wqkv, A_wo, B_w_gate.T, B_w_up.T, B_w_down, c, w_mod)
    return out.reshape(1, S, D)
```
